```python
import os as _os
_os.environ.setdefault("JAX_PLATFORMS", "cpu")
import jax
import jax.numpy as jnp

def _softmax(x, axis=-1):
    return jax.nn.softmax(x, axis=axis)
def _gelu(x):
    return jax.nn.gelu(x, approximate=True)
def _silu(x):
    return jax.nn.silu(x)
def _sigmoid(x):
    return jax.nn.sigmoid(x)
def _layernorm(x, axis=-1, eps=1e-5):
    m = jnp.mean(x, axis=axis, keepdims=True)
    v = jnp.var(x, axis=axis, keepdims=True)
    return (x - m) / jnp.sqrt(v + eps)
def _scatter_add(tgt, idx, src, axis=0):
    return tgt.at[idx].add(src)
def _segment_sum(src, seg, n):
    return jax.ops.segment_sum(src, seg, n)
class _Rng:
    def __init__(self, key):
        self._k = key
    def _next(self):
        self._k, sub = jax.random.split(self._k)
        return sub
    def normal(self, shape):
        return jax.random.normal(self._next(), shape, dtype=jnp.bfloat16)
    def randint(self, lo, hi, shape):
        return jax.random.randint(self._next(), shape, lo, hi, dtype=jnp.int32)
    def uniform(self, shape, lo=0.0, hi=1.0):
        return jax.random.uniform(self._next(), shape, jnp.bfloat16, lo, hi)
    def permutation(self, n):
        return jax.random.permutation(self._next(), n)


kernel_name = 'gated_mix__ssm_conv_s5__geglu_ffn__prompt'

def setup_inputs():
    _rng = _Rng(jax.random.key(int.from_bytes(__import__("os").urandom(4), "little")))
    _w = (lambda a: (lambda t: t.astype(jnp.bfloat16) if jnp.issubdtype(t.dtype, jnp.floating) else t)(jnp.asarray(a)))
    def _A_setup():
        B, S, D = 1, 2048, 512
        P = D
        Lambda_re = -0.5 * jnp.exp((lambda *s: _rng.normal(s) * 0.4)(P))
        Lambda_im = (lambda *s: _rng.normal(s) * 0.4)(P) * 1.0
        B_re = (lambda *s: _rng.normal(s) * 0.4)(P, D) * (D ** -0.5)
        B_im = (lambda *s: _rng.normal(s) * 0.4)(P, D) * (D ** -0.5)
        C_re = (lambda *s: _rng.normal(s) * 0.4)(D, P) * (P ** -0.5)
        C_im = (lambda *s: _rng.normal(s) * 0.4)(D, P) * (P ** -0.5)
        log_dt = (lambda *s: _rng.normal(s) * 0.4)(P) * 0.3 - 2.0
        Dskip = (lambda *s: _rng.normal(s) * 0.4)(D)
        return {
            "x": _w((lambda *s: _rng.normal(s) * 0.05)(B, S, D)),
            "Lambda_re": _w(Lambda_re),
            "Lambda_im": _w(Lambda_im),
            "B_re": _w(B_re),
            "B_im": _w(B_im),
            "C_re": _w(C_re),
            "C_im": _w(C_im),
            "log_dt": _w(log_dt),
            "Dskip": _w(Dskip),
        }
    _A_in = _A_setup()

    def _B_setup():
        B, S, D, F = 1, 2048, 512, 1376
        return {
            "x": _w((lambda *s: _rng.normal(s) * 0.05)(B, S, D)),
            "w_gate": _w((lambda *s: _rng.normal(s) * 0.1)(D, F)),
            "w_up": _w((lambda *s: _rng.normal(s) * 0.1)(D, F)),
            "w_down": _w((lambda *s: _rng.normal(s) * 0.1)(F, D)),
        }
    _B_in = _B_setup()

    return {
        "A_x": _A_in["x"],
        "A_Lambda_re": _A_in["Lambda_re"],
        "A_Lambda_im": _A_in["Lambda_im"],
        "A_B_re": _A_in["B_re"],
        "A_B_im": _A_in["B_im"],
        "A_C_re": _A_in["C_re"],
        "A_C_im": _A_in["C_im"],
        "A_log_dt": _A_in["log_dt"],
        "A_Dskip": _A_in["Dskip"],
        "B_x": _B_in["x"],
        "B_w_gate": _B_in["w_gate"],
        "B_w_up": _B_in["w_up"],
        "B_w_down": _B_in["w_down"],
        "gate_w": _w((lambda *s: _rng.normal(s) * 0.05)(512) * 16.0),
    }

def reference(A_x, A_Lambda_re, A_Lambda_im, A_B_re, A_B_im, A_C_re, A_C_im, A_log_dt, A_Dskip, B_x, B_w_gate, B_w_up, B_w_down, gate_w):
    def _A_ref(x, Lambda_re, Lambda_im, B_re, B_im, C_re, C_im, log_dt, Dskip):
        Bsz, L, H = x.shape
        Lam = Lambda_re + 1j * Lambda_im
        Bmat = B_re + 1j * B_im
        Cmat = C_re + 1j * C_im
        dt = jnp.exp(log_dt)
        Lam_bar = jnp.exp(dt * Lam)
        B_bar = ((Lam_bar - 1.0) / Lam)[:, None] * Bmat
        Bu = jnp.einsum("bld,pd->blp", x + 0j, B_bar)
        h = jnp.zeros_like(Bu[:, 0, :])
        hs = []
        for t in range(L):
            h = Lam_bar[None, :] * h + Bu[:, t, :]
            hs.append(h)
        hseq = jnp.stack(hs, 1)
        y = 2.0 * jnp.einsum("blp,dp->bld", hseq, Cmat).real + x * Dskip[None, None, :]
        return y

    def _B_ref(x, w_gate, w_up, w_down):
        return (_gelu(x @ w_gate) * (x @ w_up)) @ w_down

    x = A_x
    g = _sigmoid((x * gate_w).sum(-1, keepdims=True))
    a = _A_ref(x, A_Lambda_re, A_Lambda_im, A_B_re, A_B_im, A_C_re, A_C_im, A_log_dt, A_Dskip)
    b = _B_ref(x, B_w_gate, B_w_up, B_w_down)
    return g * a + (1 - g) * b
```

```python
import functools

import jax
import jax.numpy as jnp
from jax import lax
import jax.experimental.pallas as pl
import jax.experimental.pallas.tpu as pltpu

_NT = (((1,), (1,)), ((), ()))
_NN = (((1,), (0,)), ((), ()))


def _kernel(x_ref, lre_ref, lim_ref, bre_ref, bim_ref, cre_ref, cim_ref,
            ldt_ref, dsk_ref, wg_ref, wu_ref, wd_ref, gw_ref,
            o_ref,
            bu_re, bu_im, par, carry, seg,
            *, T, NSEG):
    S = T // NSEG
    P = par.shape[1]
    step = pl.program_id(0)

    @pl.when(step == 0)
    def _():
        lre = lre_ref[...].astype(jnp.float32)
        lim = lim_ref[...].astype(jnp.float32)
        dt = jnp.exp(ldt_ref[...].astype(jnp.float32)).astype(jnp.bfloat16).astype(jnp.float32)
        ere = jnp.exp(dt * lre)
        ang = dt * lim
        a_re = ere * jnp.cos(ang)
        a_im = ere * jnp.sin(ang)
        n_re = a_re - 1.0
        n_im = a_im
        big = jnp.abs(lre) >= jnp.abs(lim)
        r = jnp.where(big, lim / lre, lre / lim)
        den = jnp.where(big, lre + lim * r, lre * r + lim)
        f_re = jnp.where(big, (n_re + n_im * r) / den, (n_re * r + n_im) / den)
        f_im = jnp.where(big, (n_im - n_re * r) / den, (n_im * r - n_re) / den)
        p_re, p_im = a_re, a_im
        k = 1
        while k < S:
            p_re, p_im = p_re * p_re - p_im * p_im, 2.0 * p_re * p_im
            k *= 2
        par[0:1, :] = a_re
        par[1:2, :] = a_im
        par[2:3, :] = f_re
        par[3:4, :] = f_im
        par[4:5, :] = p_re
        par[5:6, :] = p_im
        par[6:8, :] = jnp.zeros((2, P), jnp.float32)
        carry[...] = jnp.zeros(carry.shape, jnp.float32)

    x = x_ref[0]

    xb_re = lax.dot_general(x, bre_ref[...], _NT, preferred_element_type=jnp.float32)
    xb_im = lax.dot_general(x, bim_ref[...], _NT, preferred_element_type=jnp.float32)
    f_re = par[2:3, :]
    f_im = par[3:4, :]
    v_re = f_re * xb_re - f_im * xb_im
    v_im = f_re * xb_im + f_im * xb_re
    G = P // 128
    for g in range(G):
        bu_re[g] = v_re[:, g * 128:(g + 1) * 128]
        bu_im[g] = v_im[:, g * 128:(g + 1) * 128]

    a_re = jnp.broadcast_to(par[0:1, :], (NSEG, P))
    a_im = jnp.broadcast_to(par[1:2, :], (NSEG, P))

    def ld(ref, k):
        return jnp.concatenate(
            [ref[g, pl.ds(k, NSEG, stride=S), :] for g in range(G)], axis=1)

    def st(ref, k, v):
        for g in range(G):
            ref[g, pl.ds(k, NSEG, stride=S), :] = v[:, g * 128:(g + 1) * 128]

    def body1(k, c):
        h_re, h_im = c
        u_re = ld(bu_re, k)
        u_im = ld(bu_im, k)
        return (a_re * h_re - a_im * h_im + u_re,
                a_re * h_im + a_im * h_re + u_im)

    z = jnp.zeros((NSEG, P), jnp.float32)
    e_re, e_im = lax.fori_loop(0, S, body1, (z, z), unroll=8)
    seg[0:NSEG, :] = e_re
    seg[NSEG:2 * NSEG, :] = e_im

    p_re = par[4:5, :]
    p_im = par[5:6, :]
    c_re = carry[0:1, :]
    c_im = carry[1:2, :]
    for j in range(NSEG):
        er = seg[j:j + 1, :]
        ei = seg[NSEG + j:NSEG + j + 1, :]
        seg[2 * NSEG + j:2 * NSEG + j + 1, :] = c_re
        seg[3 * NSEG + j:3 * NSEG + j + 1, :] = c_im
        c_re, c_im = (p_re * c_re - p_im * c_im + er,
                      p_re * c_im + p_im * c_re + ei)
    carry[0:1, :] = c_re
    carry[1:2, :] = c_im

    def body2(k, c):
        h_re, h_im = c
        u_re = ld(bu_re, k)
        u_im = ld(bu_im, k)
        n_re = a_re * h_re - a_im * h_im + u_re
        n_im = a_re * h_im + a_im * h_re + u_im
        st(bu_re, k, n_re)
        st(bu_im, k, n_im)
        return n_re, n_im

    h0_re = seg[2 * NSEG:3 * NSEG, :]
    h0_im = seg[3 * NSEG:4 * NSEG, :]
    lax.fori_loop(0, S, body2, (h0_re, h0_im), unroll=8)

    hr = jnp.concatenate([bu_re[g] for g in range(G)], axis=1).astype(jnp.bfloat16)
    hi = jnp.concatenate([bu_im[g] for g in range(G)], axis=1).astype(jnp.bfloat16)
    yc = (lax.dot_general(hr, cre_ref[...], _NT, preferred_element_type=jnp.float32)
          - lax.dot_general(hi, cim_ref[...], _NT, preferred_element_type=jnp.float32))
    xf = x.astype(jnp.float32)
    a = 2.0 * yc + xf * dsk_ref[...].astype(jnp.float32)

    gt = lax.dot_general(x, wg_ref[...], _NN, preferred_element_type=jnp.float32)
    up = lax.dot_general(x, wu_ref[...], _NN, preferred_element_type=jnp.float32)
    hid = (jax.nn.gelu(gt, approximate=True) * up).astype(jnp.bfloat16)
    b = lax.dot_general(hid, wd_ref[...], _NN, preferred_element_type=jnp.float32)

    gl = jnp.sum(xf * gw_ref[...].astype(jnp.float32), axis=-1, keepdims=True)
    g = jax.nn.sigmoid(gl)
    o_ref[0] = g * a + (1.0 - g) * b


@jax.jit
def pallas_gated_mix__ssm_conv_s5__geglu_ffn__prompt_kernel(
    A_x: jax.Array,
    A_Lambda_re: jax.Array,
    A_Lambda_im: jax.Array,
    A_B_re: jax.Array,
    A_B_im: jax.Array,
    A_C_re: jax.Array,
    A_C_im: jax.Array,
    A_log_dt: jax.Array,
    A_Dskip: jax.Array,
    B_x: jax.Array,
    B_w_gate: jax.Array,
    B_w_up: jax.Array,
    B_w_down: jax.Array,
    gate_w: jax.Array,
):
    Bsz, L, D = A_x.shape
    P = A_B_re.shape[0]
    F = B_w_gate.shape[1]
    assert Bsz == 1
    T = 512
    NSEG = 8
    assert L % T == 0

    row = lambda v: v.reshape(1, -1)
    full = lambda shape: pl.BlockSpec(shape, lambda i: (0,) * len(shape))

    kernel = functools.partial(_kernel, T=T, NSEG=NSEG)
    return pl.pallas_call(
        kernel,
        grid=(L // T,),
        in_specs=[
            pl.BlockSpec((1, T, D), lambda i: (0, i, 0)),
            full((1, P)), full((1, P)),
            full((P, D)), full((P, D)),
            full((D, P)), full((D, P)),
            full((1, P)), full((1, D)),
            full((D, F)), full((D, F)), full((F, D)),
            full((1, D)),
        ],
        out_specs=pl.BlockSpec((1, T, D), lambda i: (0, i, 0)),
        out_shape=jax.ShapeDtypeStruct((Bsz, L, D), jnp.float32),
        scratch_shapes=[
            pltpu.VMEM((P // 128, T, 128), jnp.float32),
            pltpu.VMEM((P // 128, T, 128), jnp.float32),
            pltpu.VMEM((8, P), jnp.float32),
            pltpu.VMEM((8, P), jnp.float32),
            pltpu.VMEM((4 * NSEG, P), jnp.float32),
        ],
        compiler_params=pltpu.CompilerParams(
            dimension_semantics=("arbitrary",),
            vmem_limit_bytes=100 * 1024 * 1024,
        ),
    )(A_x, row(A_Lambda_re), row(A_Lambda_im), A_B_re, A_B_im, A_C_re, A_C_im,
      row(A_log_dt), row(A_Dskip), B_w_gate, B_w_up, B_w_down, row(gate_w))
```

```python
import functools

import jax
import jax.numpy as jnp
from jax import lax
import jax.experimental.pallas as pl
import jax.experimental.pallas.tpu as pltpu

_NT = (((1,), (1,)), ((), ()))
_NN = (((1,), (0,)), ((), ()))


def _kernel(x_ref, lre_ref, lim_ref, bre_ref, bim_ref, cre_ref, cim_ref,
            ldt_ref, dsk_ref, wg_ref, wu_ref, wd_ref, gw_ref,
            o_ref,
            bu_re, bu_im, par, carry, seg,
            *, T, NSEG):
    S = T // NSEG
    P = par.shape[1]
    step = pl.program_id(0)

    @pl.when(step == 0)
    def _():
        lre = lre_ref[...].astype(jnp.float32)
        lim = lim_ref[...].astype(jnp.float32)
        dt = jnp.exp(ldt_ref[...].astype(jnp.float32)).astype(jnp.bfloat16).astype(jnp.float32)
        ere = jnp.exp(dt * lre)
        ang = dt * lim
        a_re = ere * jnp.cos(ang)
        a_im = ere * jnp.sin(ang)
        n_re = a_re - 1.0
        n_im = a_im
        big = jnp.abs(lre) >= jnp.abs(lim)
        r = jnp.where(big, lim / lre, lre / lim)
        den = jnp.where(big, lre + lim * r, lre * r + lim)
        f_re = jnp.where(big, (n_re + n_im * r) / den, (n_re * r + n_im) / den)
        f_im = jnp.where(big, (n_im - n_re * r) / den, (n_im * r - n_re) / den)
        p_re, p_im = a_re, a_im
        k = 1
        while k < S:
            p_re, p_im = p_re * p_re - p_im * p_im, 2.0 * p_re * p_im
            k *= 2
        par[0:1, :] = a_re
        par[1:2, :] = a_im
        par[2:3, :] = f_re
        par[3:4, :] = f_im
        par[4:5, :] = p_re
        par[5:6, :] = p_im
        par[6:8, :] = jnp.zeros((2, P), jnp.float32)
        carry[...] = jnp.zeros(carry.shape, jnp.float32)

    x = x_ref[0]

    xb_re = lax.dot_general(x, bre_ref[...], _NT, preferred_element_type=jnp.float32)
    xb_im = lax.dot_general(x, bim_ref[...], _NT, preferred_element_type=jnp.float32)
    f_re = par[2:3, :]
    f_im = par[3:4, :]
    v_re = f_re * xb_re - f_im * xb_im
    v_im = f_re * xb_im + f_im * xb_re
    G = P // 128
    for g in range(G):
        bu_re[g] = v_re[:, g * 128:(g + 1) * 128]
        bu_im[g] = v_im[:, g * 128:(g + 1) * 128]

    a_re = jnp.broadcast_to(par[0:1, :], (NSEG, P))
    a_im = jnp.broadcast_to(par[1:2, :], (NSEG, P))

    def ld(ref, k):
        return jnp.concatenate(
            [ref[g, pl.ds(k, NSEG, stride=S), :] for g in range(G)], axis=1)

    def st(ref, k, v):
        for g in range(G):
            ref[g, pl.ds(k, NSEG, stride=S), :] = v[:, g * 128:(g + 1) * 128]

    def body1(k, c):
        h_re, h_im = c
        u_re = ld(bu_re, k)
        u_im = ld(bu_im, k)
        return (a_re * h_re - a_im * h_im + u_re,
                a_re * h_im + a_im * h_re + u_im)

    z = jnp.zeros((NSEG, P), jnp.float32)
    e_re, e_im = lax.fori_loop(0, S, body1, (z, z), unroll=8)
    seg[0:NSEG, :] = e_re
    seg[NSEG:2 * NSEG, :] = e_im

    p_re = par[4:5, :]
    p_im = par[5:6, :]
    c_re = carry[0:1, :]
    c_im = carry[1:2, :]
    for j in range(NSEG):
        er = seg[j:j + 1, :]
        ei = seg[NSEG + j:NSEG + j + 1, :]
        seg[2 * NSEG + j:2 * NSEG + j + 1, :] = c_re
        seg[3 * NSEG + j:3 * NSEG + j + 1, :] = c_im
        c_re, c_im = (p_re * c_re - p_im * c_im + er,
                      p_re * c_im + p_im * c_re + ei)
    carry[0:1, :] = c_re
    carry[1:2, :] = c_im

    def body2(k, c):
        h_re, h_im = c
        u_re = ld(bu_re, k)
        u_im = ld(bu_im, k)
        n_re = a_re * h_re - a_im * h_im + u_re
        n_im = a_re * h_im + a_im * h_re + u_im
        st(bu_re, k, n_re)
        st(bu_im, k, n_im)
        return n_re, n_im

    h0_re = seg[2 * NSEG:3 * NSEG, :]
    h0_im = seg[3 * NSEG:4 * NSEG, :]
    lax.fori_loop(0, S, body2, (h0_re, h0_im), unroll=8)

    hr = jnp.concatenate([bu_re[g] for g in range(G)], axis=1).astype(jnp.bfloat16)
    hi = jnp.concatenate([bu_im[g] for g in range(G)], axis=1).astype(jnp.bfloat16)
    yc = (lax.dot_general(hr, cre_ref[...], _NT, preferred_element_type=jnp.float32)
          - lax.dot_general(hi, cim_ref[...], _NT, preferred_element_type=jnp.float32))
    xf = x.astype(jnp.float32)
    a = 2.0 * yc + xf * dsk_ref[...].astype(jnp.float32)

    gt = lax.dot_general(x, wg_ref[...], _NT, preferred_element_type=jnp.float32)
    up = lax.dot_general(x, wu_ref[...], _NT, preferred_element_type=jnp.float32)
    hid = (jax.nn.gelu(gt, approximate=True) * up).astype(jnp.bfloat16)
    b = lax.dot_general(hid, wd_ref[...], _NN, preferred_element_type=jnp.float32)

    gl = jnp.sum(xf * gw_ref[...].astype(jnp.float32), axis=-1, keepdims=True)
    g = jax.nn.sigmoid(gl)
    o_ref[0] = g * a + (1.0 - g) * b


@jax.jit
def pallas_gated_mix__ssm_conv_s5__geglu_ffn__prompt_kernel(
    A_x: jax.Array,
    A_Lambda_re: jax.Array,
    A_Lambda_im: jax.Array,
    A_B_re: jax.Array,
    A_B_im: jax.Array,
    A_C_re: jax.Array,
    A_C_im: jax.Array,
    A_log_dt: jax.Array,
    A_Dskip: jax.Array,
    B_x: jax.Array,
    B_w_gate: jax.Array,
    B_w_up: jax.Array,
    B_w_down: jax.Array,
    gate_w: jax.Array,
):
    Bsz, L, D = A_x.shape
    P = A_B_re.shape[0]
    F = B_w_gate.shape[1]
    assert Bsz == 1
    T = 512
    NSEG = 8
    assert L % T == 0

    row = lambda v: v.reshape(1, -1)
    full = lambda shape: pl.BlockSpec(shape, lambda i: (0,) * len(shape))

    kernel = functools.partial(_kernel, T=T, NSEG=NSEG)
    return pl.pallas_call(
        kernel,
        grid=(L // T,),
        in_specs=[
            pl.BlockSpec((1, T, D), lambda i: (0, i, 0)),
            full((1, P)), full((1, P)),
            full((P, D)), full((P, D)),
            full((D, P)), full((D, P)),
            full((1, P)), full((1, D)),
            full((F, D)), full((F, D)), full((F, D)),
            full((1, D)),
        ],
        out_specs=pl.BlockSpec((1, T, D), lambda i: (0, i, 0)),
        out_shape=jax.ShapeDtypeStruct((Bsz, L, D), jnp.float32),
        scratch_shapes=[
            pltpu.VMEM((P // 128, T, 128), jnp.float32),
            pltpu.VMEM((P // 128, T, 128), jnp.float32),
            pltpu.VMEM((8, P), jnp.float32),
            pltpu.VMEM((8, P), jnp.float32),
            pltpu.VMEM((4 * NSEG, P), jnp.float32),
        ],
        compiler_params=pltpu.CompilerParams(
            dimension_semantics=("arbitrary",),
            vmem_limit_bytes=100 * 1024 * 1024,
        ),
    )(A_x, row(A_Lambda_re), row(A_Lambda_im), A_B_re, A_B_im, A_C_re, A_C_im,
      row(A_log_dt), row(A_Dskip), B_w_gate.T, B_w_up.T, B_w_down, row(gate_w))
```

```python
import functools

import jax
import jax.numpy as jnp
from jax import lax
import jax.experimental.pallas as pl
import jax.experimental.pallas.tpu as pltpu

_NT = (((1,), (1,)), ((), ()))
_NN = (((1,), (0,)), ((), ()))


def _cmul(ar, ai, br, bi):
    return ar * br - ai * bi, ar * bi + ai * br


def _kernel(xc_ref, xp_ref, lre_ref, lim_ref, bre_ref, bim_ref, cre_hbm, cim_hbm,
            ldt_ref, dsk_ref, wg_hbm, wu_hbm, wd_hbm, gw_ref,
            o_hbm,
            h_re_s, h_im_s, hid_s, ya_s, par, carry,
            cre_ref, cim_ref, wg_ref, wu_ref, wd_ref, o_buf, sems, osems,
            *, T, NT):
    P = par.shape[-1]
    F = wg_ref.shape[0]
    step = pl.program_id(0)
    nchunk = (F + 127) // 128
    nblk = T // 8

    copies = [
        pltpu.make_async_copy(src, dst, sems.at[i])
        for i, (src, dst) in enumerate((
            (cre_hbm, cre_ref), (cim_hbm, cim_ref),
            (wg_hbm, wg_ref), (wu_hbm, wu_ref), (wd_hbm, wd_ref)))
    ]

    NCH = 4
    RC = T // NCH

    def out_copy(tile, slot, ch):
        return pltpu.make_async_copy(
            o_buf.at[slot, pl.ds(ch * RC, RC), :],
            o_hbm.at[0, pl.ds(pl.multiple_of(tile * T, T) + ch * RC, RC), :],
            osems.at[slot, ch])

    def params():
        lre = lre_ref[...].astype(jnp.float32).reshape(1, P)
        lim = lim_ref[...].astype(jnp.float32).reshape(1, P)
        dt = jnp.exp(ldt_ref[...].astype(jnp.float32).reshape(1, P)).astype(jnp.bfloat16).astype(jnp.float32)
        ere = jnp.exp(dt * lre)
        ang = dt * lim
        a_re = ere * jnp.cos(ang)
        a_im = ere * jnp.sin(ang)
        n_re = a_re - 1.0
        n_im = a_im
        big = jnp.abs(lre) >= jnp.abs(lim)
        r = jnp.where(big, lim / lre, lre / lim)
        den = jnp.where(big, lre + lim * r, lre * r + lim)
        f_re = jnp.where(big, (n_re + n_im * r) / den, (n_re * r + n_im) / den)
        f_im = jnp.where(big, (n_im - n_re * r) / den, (n_im * r - n_re) / den)
        par[0, :, :] = jnp.broadcast_to(f_re, (8, P))
        par[1, :, :] = jnp.broadcast_to(f_im, (8, P))
        pw = [(a_re, a_im)]
        for _k in range(7):
            pw.append(_cmul(pw[-1][0], pw[-1][1], a_re, a_im))
        row = lax.broadcasted_iota(jnp.int32, (8, P), 0)
        for idx, d in enumerate((1, 2, 4)):
            par[2 + 2 * idx, :, :] = jnp.where(row >= d, pw[d - 1][0], 0.0)
            par[3 + 2 * idx, :, :] = jnp.where(row >= d, pw[d - 1][1], 0.0)
        cr = jnp.zeros((8, P), jnp.float32)
        ci = jnp.zeros((8, P), jnp.float32)
        for j in range(8):
            cr = jnp.where(row == j, pw[j][0], cr)
            ci = jnp.where(row == j, pw[j][1], ci)
        par[8, :, :] = cr
        par[9, :, :] = ci
        carry[...] = jnp.zeros(carry.shape, jnp.float32)

    def compute(do_ssm, do_ffn, first):
        if do_ssm:
            xc = xc_ref[0]
            xb_re = lax.dot_general(xc, bre_ref[...], _NT, preferred_element_type=jnp.float32)
            xb_im = lax.dot_general(xc, bim_ref[...], _NT, preferred_element_type=jnp.float32)
            f_re = par[0]
            f_im = par[1]
            coef = [(par[2 + 2 * i], par[3 + 2 * i]) for i in range(3)]
            cw_re = par[8]
            cw_im = par[9]
            c_re = carry[0]
            c_im = carry[1]

        def scan_rows(m0, m1, fj_re, fj_im, c_re, c_im):
            for m in range(m0, m1):
                sl = slice(m * 8, (m + 1) * 8)
                v_re, v_im = _cmul(fj_re, fj_im, xb_re[sl], xb_im[sl])
                for (d, (k_re, k_im)) in zip((1, 2, 4), coef):
                    s_re = pltpu.roll(v_re, d, 0)
                    s_im = pltpu.roll(v_im, d, 0)
                    t_re, t_im = _cmul(k_re, k_im, s_re, s_im)
                    v_re = v_re + t_re
                    v_im = v_im + t_im
                t_re, t_im = _cmul(cw_re, cw_im, c_re, c_im)
                v_re = v_re + t_re
                v_im = v_im + t_im
                h_re_s[sl, :] = v_re.astype(jnp.bfloat16)
                h_im_s[sl, :] = v_im.astype(jnp.bfloat16)
                c_re = jnp.broadcast_to(v_re[7:8, :], (8, P))
                c_im = jnp.broadcast_to(v_im[7:8, :], (8, P))
            return c_re, c_im

        m = 0
        if do_ssm and not do_ffn:
            c_re, c_im = scan_rows(0, nblk, f_re, f_im, c_re, c_im)
            m = nblk
        if do_ffn:
            x = xp_ref[0]
            for j in range(nchunk):
                lo, hi = j * 128, min(F, (j + 1) * 128)
                gt = lax.dot_general(x, wg_ref[lo:hi, :], _NT, preferred_element_type=jnp.float32)
                up = lax.dot_general(x, wu_ref[lo:hi, :], _NT, preferred_element_type=jnp.float32)
                hid_s[:, lo:hi] = (jax.nn.gelu(gt, approximate=True) * up).astype(jnp.bfloat16)
                m_end = min(nblk, (nblk * (j + 1)) // (nchunk - 4)) if do_ssm else 0
                if m < m_end:
                    tie = jnp.concatenate([up[T - 8:T, 0:128]] * (P // 128), axis=1)
                    fj_re = jnp.where(step < 0, tie, f_re)
                    fj_im = jnp.where(step < 0, tie, f_im)
                    c_re, c_im = scan_rows(m, m_end, fj_re, fj_im, c_re, c_im)
                    m = m_end
            slot = (step + 1) % 2
            dsk = dsk_ref[...].astype(jnp.float32).reshape(1, -1)
            gw = gw_ref[...].astype(jnp.float32).reshape(1, -1)
            for ch in range(NCH if not do_ssm else 1):
                rows = slice(ch * RC, (ch + 1) * RC) if not do_ssm else slice(0, T)
                b = lax.dot_general(hid_s[rows, :], wd_ref[...], _NN, preferred_element_type=jnp.float32)
                xf = x[rows].astype(jnp.float32)
                a = ya_s[slot, rows, :] + xf * dsk
                gl = jnp.sum(xf * gw, axis=-1, keepdims=True)
                g = jax.nn.sigmoid(gl)
                o_buf[slot, rows, :] = g * a + (1.0 - g) * b
                if not do_ssm:
                    out_copy(step - 1, slot, ch).start()
            if do_ssm:
                for ch in range(NCH):
                    out_copy(step - 1, slot, ch).start()
        if do_ssm:
            carry[0] = c_re
            carry[1] = c_im
            if first:
                copies[0].wait()
                copies[1].wait()
            yc = (lax.dot_general(h_re_s[...], cre_ref[...], _NT, preferred_element_type=jnp.float32)
                  - lax.dot_general(h_im_s[...], cim_ref[...], _NT, preferred_element_type=jnp.float32))
            ya_s[step % 2] = 2.0 * yc

    @pl.when(step == 0)
    def _():
        for c in copies:
            c.start()
        params()
        compute(True, False, True)

    @pl.when(step == 1)
    def _():
        for c in copies[2:]:
            c.wait()

    @pl.when(step >= 3)
    def _():
        for ch in range(NCH):
            out_copy(step - 3, (step + 1) % 2, ch).wait()

    @pl.when(jnp.logical_and(step > 0, step < NT))
    def _():
        compute(True, True, False)

    @pl.when(step == NT)
    def _():
        compute(False, True, False)
        if NT >= 2:
            for ch in range(NCH):
                out_copy(step - 2, step % 2, ch).wait()
        for ch in range(NCH):
            out_copy(step - 1, (step + 1) % 2, ch).wait()


@jax.jit
def pallas_gated_mix__ssm_conv_s5__geglu_ffn__prompt_kernel(
    A_x: jax.Array,
    A_Lambda_re: jax.Array,
    A_Lambda_im: jax.Array,
    A_B_re: jax.Array,
    A_B_im: jax.Array,
    A_C_re: jax.Array,
    A_C_im: jax.Array,
    A_log_dt: jax.Array,
    A_Dskip: jax.Array,
    B_x: jax.Array,
    B_w_gate: jax.Array,
    B_w_up: jax.Array,
    B_w_down: jax.Array,
    gate_w: jax.Array,
):
    Bsz, L, D = A_x.shape
    P = A_B_re.shape[0]
    F = B_w_gate.shape[1]
    assert Bsz == 1
    T = 512
    assert L % T == 0
    NT = L // T

    full = lambda shape: pl.BlockSpec(shape, lambda i: (0,) * len(shape))
    hbm = pl.BlockSpec(memory_space=pl.ANY)

    kernel = functools.partial(_kernel, T=T, NT=NT)
    return pl.pallas_call(
        kernel,
        grid=(NT + 1,),
        in_specs=[
            pl.BlockSpec((1, T, D), lambda i: (0, jnp.minimum(i, NT - 1), 0)),
            pl.BlockSpec((1, T, D), lambda i: (0, jnp.maximum(i - 1, 0), 0)),
            full((P,)), full((P,)),
            full((P, D)), full((P, D)),
            hbm, hbm,
            full((P,)), full((D,)),
            hbm, hbm, hbm,
            full((D,)),
        ],
        out_specs=hbm,
        out_shape=jax.ShapeDtypeStruct((Bsz, L, D), jnp.float32),
        scratch_shapes=[
            pltpu.VMEM((T, P), jnp.bfloat16),
            pltpu.VMEM((T, P), jnp.bfloat16),
            pltpu.VMEM((T, F), jnp.bfloat16),
            pltpu.VMEM((2, T, D), jnp.float32),
            pltpu.VMEM((10, 8, P), jnp.float32),
            pltpu.VMEM((2, 8, P), jnp.float32),
            pltpu.VMEM((D, P), jnp.bfloat16),
            pltpu.VMEM((D, P), jnp.bfloat16),
            pltpu.VMEM((F, D), jnp.bfloat16),
            pltpu.VMEM((F, D), jnp.bfloat16),
            pltpu.VMEM((F, D), jnp.bfloat16),
            pltpu.VMEM((2, T, D), jnp.float32),
            pltpu.SemaphoreType.DMA((5,)),
            pltpu.SemaphoreType.DMA((2, 4)),
        ],
        compiler_params=pltpu.CompilerParams(
            dimension_semantics=("arbitrary",),
            vmem_limit_bytes=100 * 1024 * 1024,
        ),
    )(A_x, A_x, A_Lambda_re, A_Lambda_im, A_B_re, A_B_im, A_C_re, A_C_im,
      A_log_dt, A_Dskip, B_w_gate.T, B_w_up.T, B_w_down, gate_w)
```

```python
import functools

import jax
import jax.numpy as jnp
from jax import lax
import jax.experimental.pallas as pl
import jax.experimental.pallas.tpu as pltpu

_NT = (((1,), (1,)), ((), ()))
_NN = (((1,), (0,)), ((), ()))


def _bf(v):
    return v.astype(jnp.bfloat16).astype(jnp.float32)


def _cmul(ar, ai, br, bi):
    return ar * br - ai * bi, ar * bi + ai * br


def _kernel(xc_ref, xp_ref, lre_ref, lim_ref, bre_ref, bim_ref, cre_hbm, cim_hbm,
            ldt_ref, dsk_ref, wg_hbm, wu_hbm, wd_hbm, gw_ref,
            o_hbm,
            h_re_s, h_im_s, hid_s, ya_s, par, carry,
            cre_ref, cim_ref, wg_ref, wu_ref, wd_ref, o_buf, sems, osems,
            *, T, NT):
    P = par.shape[-1]
    F = wg_ref.shape[0]
    step = pl.program_id(0)
    nchunk = (F + 127) // 128
    nblk = T // 8

    copies = [
        pltpu.make_async_copy(src, dst, sems.at[i])
        for i, (src, dst) in enumerate((
            (cre_hbm, cre_ref), (cim_hbm, cim_ref),
            (wg_hbm, wg_ref), (wu_hbm, wu_ref), (wd_hbm, wd_ref)))
    ]

    NCH = 4
    RC = T // NCH

    def out_copy(tile, slot, ch):
        return pltpu.make_async_copy(
            o_buf.at[slot, pl.ds(ch * RC, RC), :],
            o_hbm.at[0, pl.ds(pl.multiple_of(tile * T, T) + ch * RC, RC), :],
            osems.at[slot, ch])

    def params():
        lre = lre_ref[...].astype(jnp.float32).reshape(1, P)
        lim = lim_ref[...].astype(jnp.float32).reshape(1, P)
        dt = jnp.exp(ldt_ref[...].astype(jnp.float32).reshape(1, P)).astype(jnp.bfloat16).astype(jnp.float32)
        ere = jnp.exp(dt * lre)
        ang = dt * lim
        a_re = ere * jnp.cos(ang)
        a_im = ere * jnp.sin(ang)
        n_re = a_re - 1.0
        n_im = a_im
        big = jnp.abs(lre) >= jnp.abs(lim)
        r = jnp.where(big, lim / lre, lre / lim)
        den = jnp.where(big, lre + lim * r, lre * r + lim)
        f_re = jnp.where(big, (n_re + n_im * r) / den, (n_re * r + n_im) / den)
        f_im = jnp.where(big, (n_im - n_re * r) / den, (n_im * r - n_re) / den)
        par[0, :, :] = jnp.broadcast_to(f_re, (8, P))
        par[1, :, :] = jnp.broadcast_to(f_im, (8, P))
        pw = [(a_re, a_im)]
        for _k in range(7):
            pw.append(_cmul(pw[-1][0], pw[-1][1], a_re, a_im))
        row = lax.broadcasted_iota(jnp.int32, (8, P), 0)
        for idx, d in enumerate((1, 2, 4)):
            par[2 + 2 * idx, :, :] = jnp.where(row >= d, pw[d - 1][0], 0.0)
            par[3 + 2 * idx, :, :] = jnp.where(row >= d, pw[d - 1][1], 0.0)
        cr = jnp.zeros((8, P), jnp.float32)
        ci = jnp.zeros((8, P), jnp.float32)
        for j in range(8):
            cr = jnp.where(row == j, pw[j][0], cr)
            ci = jnp.where(row == j, pw[j][1], ci)
        par[8, :, :] = cr
        par[9, :, :] = ci
        carry[...] = jnp.zeros(carry.shape, jnp.float32)

    def compute(do_ssm, do_ffn, first):
        if do_ssm:
            xc = xc_ref[0]
            xb_re = lax.dot_general(xc, bre_ref[...], _NT, preferred_element_type=jnp.float32)
            xb_im = lax.dot_general(xc, bim_ref[...], _NT, preferred_element_type=jnp.float32)
            f_re = par[0]
            f_im = par[1]
            coef = [(par[2 + 2 * i], par[3 + 2 * i]) for i in range(3)]
            cw_re = par[8]
            cw_im = par[9]
            c_re = carry[0]
            c_im = carry[1]

        def scan_rows(m0, m1, fj_re, fj_im, c_re, c_im):
            for m in range(m0, m1):
                sl = slice(m * 8, (m + 1) * 8)
                v_re, v_im = _cmul(fj_re, fj_im, xb_re[sl], xb_im[sl])
                for (d, (k_re, k_im)) in zip((1, 2, 4), coef):
                    s_re = pltpu.roll(v_re, d, 0)
                    s_im = pltpu.roll(v_im, d, 0)
                    t_re, t_im = _cmul(k_re, k_im, s_re, s_im)
                    v_re = v_re + t_re
                    v_im = v_im + t_im
                t_re, t_im = _cmul(cw_re, cw_im, c_re, c_im)
                v_re = v_re + t_re
                v_im = v_im + t_im
                h_re_s[sl, :] = v_re.astype(jnp.bfloat16)
                h_im_s[sl, :] = v_im.astype(jnp.bfloat16)
                c_re = jnp.broadcast_to(v_re[7:8, :], (8, P))
                c_im = jnp.broadcast_to(v_im[7:8, :], (8, P))
            return c_re, c_im

        m = 0
        if do_ssm and not do_ffn:
            c_re, c_im = scan_rows(0, nblk, f_re, f_im, c_re, c_im)
            m = nblk
        if do_ffn:
            x = xp_ref[0]
            for j in range(nchunk):
                lo, hi = j * 128, min(F, (j + 1) * 128)
                gt = lax.dot_general(x, wg_ref[lo:hi, :], _NT, preferred_element_type=jnp.float32)
                up = lax.dot_general(x, wu_ref[lo:hi, :], _NT, preferred_element_type=jnp.float32)
                hid_s[:, lo:hi] = (jax.nn.gelu(gt, approximate=True) * up).astype(jnp.bfloat16)
                m_end = min(nblk, (nblk * (j + 1)) // (nchunk - 4)) if do_ssm else 0
                if m < m_end:
                    tie = jnp.concatenate([up[T - 8:T, 0:128]] * (P // 128), axis=1)
                    fj_re = jnp.where(step < 0, tie, f_re)
                    fj_im = jnp.where(step < 0, tie, f_im)
                    c_re, c_im = scan_rows(m, m_end, fj_re, fj_im, c_re, c_im)
                    m = m_end
            slot = (step + 1) % 2
            dsk = dsk_ref[...].astype(jnp.float32).reshape(1, -1)
            gw = gw_ref[...].astype(jnp.float32).reshape(1, -1)
            for ch in range(NCH if not do_ssm else 1):
                rows = slice(ch * RC, (ch + 1) * RC) if not do_ssm else slice(0, T)
                b = lax.dot_general(hid_s[rows, :], wd_ref[...], _NN, preferred_element_type=jnp.float32)
                xf = x[rows].astype(jnp.float32)
                a = ya_s[slot, rows, :] + _bf(xf * dsk)
                gl = _bf(jnp.sum(_bf(xf * gw), axis=-1, keepdims=True))
                g = _bf(jax.nn.sigmoid(gl))
                o_buf[slot, rows, :] = g * a + _bf(_bf(1.0 - g) * _bf(b))
                if not do_ssm:
                    out_copy(step - 1, slot, ch).start()
            if do_ssm:
                for ch in range(NCH):
                    out_copy(step - 1, slot, ch).start()
        if do_ssm:
            carry[0] = c_re
            carry[1] = c_im
            if first:
                copies[0].wait()
                copies[1].wait()
            yc = (lax.dot_general(h_re_s[...], cre_ref[...], _NT, preferred_element_type=jnp.float32)
                  - lax.dot_general(h_im_s[...], cim_ref[...], _NT, preferred_element_type=jnp.float32))
            ya_s[step % 2] = 2.0 * yc

    @pl.when(step == 0)
    def _():
        for c in copies:
            c.start()
        params()
        compute(True, False, True)

    @pl.when(step == 1)
    def _():
        for c in copies[2:]:
            c.wait()

    @pl.when(step >= 3)
    def _():
        for ch in range(NCH):
            out_copy(step - 3, (step + 1) % 2, ch).wait()

    @pl.when(jnp.logical_and(step > 0, step < NT))
    def _():
        compute(True, True, False)

    @pl.when(step == NT)
    def _():
        compute(False, True, False)
        if NT >= 2:
            for ch in range(NCH):
                out_copy(step - 2, step % 2, ch).wait()
        for ch in range(NCH):
            out_copy(step - 1, (step + 1) % 2, ch).wait()


@jax.jit
def pallas_gated_mix__ssm_conv_s5__geglu_ffn__prompt_kernel(
    A_x: jax.Array,
    A_Lambda_re: jax.Array,
    A_Lambda_im: jax.Array,
    A_B_re: jax.Array,
    A_B_im: jax.Array,
    A_C_re: jax.Array,
    A_C_im: jax.Array,
    A_log_dt: jax.Array,
    A_Dskip: jax.Array,
    B_x: jax.Array,
    B_w_gate: jax.Array,
    B_w_up: jax.Array,
    B_w_down: jax.Array,
    gate_w: jax.Array,
):
    Bsz, L, D = A_x.shape
    P = A_B_re.shape[0]
    F = B_w_gate.shape[1]
    assert Bsz == 1
    T = 512
    assert L % T == 0
    NT = L // T

    full = lambda shape: pl.BlockSpec(shape, lambda i: (0,) * len(shape))
    hbm = pl.BlockSpec(memory_space=pl.ANY)

    kernel = functools.partial(_kernel, T=T, NT=NT)
    return pl.pallas_call(
        kernel,
        grid=(NT + 1,),
        in_specs=[
            pl.BlockSpec((1, T, D), lambda i: (0, jnp.minimum(i, NT - 1), 0)),
            pl.BlockSpec((1, T, D), lambda i: (0, jnp.maximum(i - 1, 0), 0)),
            full((P,)), full((P,)),
            full((P, D)), full((P, D)),
            hbm, hbm,
            full((P,)), full((D,)),
            hbm, hbm, hbm,
            full((D,)),
        ],
        out_specs=hbm,
        out_shape=jax.ShapeDtypeStruct((Bsz, L, D), jnp.float32),
        scratch_shapes=[
            pltpu.VMEM((T, P), jnp.bfloat16),
            pltpu.VMEM((T, P), jnp.bfloat16),
            pltpu.VMEM((T, F), jnp.bfloat16),
            pltpu.VMEM((2, T, D), jnp.float32),
            pltpu.VMEM((10, 8, P), jnp.float32),
            pltpu.VMEM((2, 8, P), jnp.float32),
            pltpu.VMEM((D, P), jnp.bfloat16),
            pltpu.VMEM((D, P), jnp.bfloat16),
            pltpu.VMEM((F, D), jnp.bfloat16),
            pltpu.VMEM((F, D), jnp.bfloat16),
            pltpu.VMEM((F, D), jnp.bfloat16),
            pltpu.VMEM((2, T, D), jnp.float32),
            pltpu.SemaphoreType.DMA((5,)),
            pltpu.SemaphoreType.DMA((2, 4)),
        ],
        compiler_params=pltpu.CompilerParams(
            dimension_semantics=("arbitrary",),
            vmem_limit_bytes=100 * 1024 * 1024,
        ),
    )(A_x, A_x, A_Lambda_re, A_Lambda_im, A_B_re, A_B_im, A_C_re, A_C_im,
      A_log_dt, A_Dskip, B_w_gate.T, B_w_up.T, B_w_down, gate_w)
```
